```python
import os as _os
_os.environ.setdefault('JAX_PLATFORMS', 'cpu')
import jax
import jax.numpy as jnp

def _softmax(x, axis=-1):
    return jax.nn.softmax(x, axis=axis)

def _gelu(x):
    return jax.nn.gelu(x, approximate=True)

def _silu(x):
    return jax.nn.silu(x)

def _sigmoid(x):
    return jax.nn.sigmoid(x)

def _layernorm(x, axis=-1, eps=1e-05):
    m = jnp.mean(x, axis=axis, keepdims=True)
    v = jnp.var(x, axis=axis, keepdims=True)
    return (x - m) / jnp.sqrt(v + eps)

def _scatter_add(tgt, idx, src, axis=0):
    return tgt.at[idx].add(src)

def _segment_sum(src, seg, n):
    return jax.ops.segment_sum(src, seg, n)

class _Rng:

    def __init__(self, key):
        self._k = key

    def _next(self):
        self._k, sub = jax.random.split(self._k)
        return sub

    def normal(self, shape):
        return jax.random.normal(self._next(), shape, dtype=jnp.bfloat16)

    def randint(self, lo, hi, shape):
        return jax.random.randint(self._next(), shape, lo, hi, dtype=jnp.int32)

    def uniform(self, shape, lo=0.0, hi=1.0):
        return jax.random.uniform(self._next(), shape, jnp.bfloat16, lo, hi)

    def permutation(self, n):
        return jax.random.permutation(self._next(), n)
kernel_name = 'gated_mix__memory_aug_recurrent_mem_tr__glu_gated_geglu__prompt'

def setup_inputs():
    _rng = _Rng(jax.random.key(int.from_bytes(__import__("os").urandom(4), "little")))
    _w = lambda a: (lambda t: t.astype(jnp.bfloat16) if jnp.issubdtype(t.dtype, jnp.floating) else t)(jnp.asarray(a))

    def _A_setup():
        B, S, Dm = (1, 2048, 640)
        H, Dh = (32, 128)
        M, seg = (8, 32)
        seg = min(seg, S)
        S = S // seg * seg
        return {'x': _w((lambda *s: _rng.normal(s) * 0.05)(B, S, Dm)), 'mem0': _w((lambda *s: _rng.normal(s) * 0.4)(B, M, Dm)), 'Wq': _w((lambda *s: _rng.normal(s) * 3.2)(Dm, H, Dh) * Dm ** (-0.5)), 'Wk': _w((lambda *s: _rng.normal(s) * 3.2)(Dm, H, Dh) * Dm ** (-0.5)), 'Wv': _w((lambda *s: _rng.normal(s) * 0.4)(Dm, H, Dh) * Dm ** (-0.5)), 'Wo': _w((lambda *s: _rng.normal(s) * 0.4)(H, Dh, Dm) * (H * Dh) ** (-0.5)), 'seg_len': seg}
    _A_in = _A_setup()

    def _B_setup():
        B, S, Dm, Df = (1, 2048, 640, 1728)
        return {'x': _w((lambda *s: _rng.normal(s) * 0.05)(B, S, Dm)), 'w_gate': _w((lambda *s: _rng.normal(s) * 1.6)(Dm, Df) * Dm ** (-0.5)), 'w_up': _w((lambda *s: _rng.normal(s) * 1.6)(Dm, Df) * Dm ** (-0.5)), 'w_down': _w((lambda *s: _rng.normal(s) * 1.6)(Df, Dm) * Df ** (-0.5))}
    _B_in = _B_setup()
    return {'A_x': _A_in['x'], 'A_mem0': _A_in['mem0'], 'A_Wq': _A_in['Wq'], 'A_Wk': _A_in['Wk'], 'A_Wv': _A_in['Wv'], 'A_Wo': _A_in['Wo'], 'A_seg_len': _A_in['seg_len'], 'B_x': _B_in['x'], 'B_w_gate': _B_in['w_gate'], 'B_w_up': _B_in['w_up'], 'B_w_down': _B_in['w_down'], 'gate_w': _w((lambda *s: _rng.normal(s) * 0.05)(640) * 16.0)}

def reference(A_x, A_mem0, A_Wq, A_Wk, A_Wv, A_Wo, A_seg_len, B_x, B_w_gate, B_w_up, B_w_down, gate_w):

    def _A_ref(x, mem0, Wq, Wk, Wv, Wo, seg_len):
        B, S, Dm = x.shape
        H, Dh = (Wq.shape[1], Wq.shape[2])
        M = mem0.shape[1]
        scale = Dh ** (-0.5)
        n_seg = S // seg_len
        L = M + seg_len
        idx = jnp.arange(L)
        mask = (idx[:, None] < M) | (idx[:, None] >= idx[None, :])
        mem = mem0
        outs = []
        for s in range(n_seg):
            xs = x[:, s * seg_len:(s + 1) * seg_len, :].copy()
            h = jnp.concatenate([mem, xs], axis=1)
            q = jnp.einsum('btd,dhe->bhte', h, Wq)
            k = jnp.einsum('btd,dhe->bhte', h, Wk)
            v = jnp.einsum('btd,dhe->bhte', h, Wv)
            scores = jnp.einsum('bhqe,bhke->bhqk', q, k) * scale
            scores = jnp.where(mask[None, None], scores, -1000000000.0)
            p = _softmax(scores, axis=-1)
            o = jnp.einsum('bhqk,bhke->bhqe', p, v)
            o = jnp.einsum('bhte,hed->btd', o, Wo)
            mem = o[:, :M, :].copy()
            outs.append(o[:, M:, :])
        return jnp.concatenate(outs, axis=1)

    def _B_ref(x, w_gate, w_up, w_down):
        g = jnp.einsum('bsd,df->bsf', x, w_gate)
        u = jnp.einsum('bsd,df->bsf', x, w_up)
        h = _gelu(g) * u
        return jnp.einsum('bsf,fd->bsd', h, w_down)
    x = A_x
    g = _sigmoid((x * gate_w).sum(-1, keepdims=True))
    a = _A_ref(x, A_mem0, A_Wq, A_Wk, A_Wv, A_Wo, A_seg_len)
    b = _B_ref(x, B_w_gate, B_w_up, B_w_down)
    return g * a + (1 - g) * b
```

```python
import functools

import jax
import jax.numpy as jnp
from jax import lax
import jax.experimental.pallas as pl
import jax.experimental.pallas.tpu as pltpu

_F32 = jnp.float32
_BF16 = jnp.bfloat16
_MC = 256


def _dot(a, b):
    return jnp.dot(a, b, preferred_element_type=_F32)


def _kernel(x_hbm, mem_hbm, wq_hbm, wk_hbm, wv_hbm, wo_hbm, wg_hbm, wu_hbm, wd_hbm, gw_hbm,
            out_hbm,
            x_v, mem_v, gw_v, wg_v, wu_v, wd_v, stage_v, w_v, wo_v, b_v, g_v, o_v,
            sem_in, sem_w, sem_out, *, seg, n_heads):
    S, Dm = x_v.shape
    M = mem_v.shape[0]
    Dh = stage_v.shape[2]
    L = M + seg
    n_seg = S // seg
    n_pair = n_heads // 2
    n_chunk = S // _MC
    scale = Dh ** (-0.5)

    small = [
        pltpu.make_async_copy(x_hbm, x_v, sem_in.at[0]),
        pltpu.make_async_copy(gw_hbm, gw_v, sem_in.at[1]),
        pltpu.make_async_copy(wg_hbm, wg_v, sem_in.at[2]),
        pltpu.make_async_copy(wu_hbm, wu_v, sem_in.at[3]),
        pltpu.make_async_copy(wd_hbm, wd_v, sem_in.at[4]),
        pltpu.make_async_copy(mem_hbm, mem_v, sem_in.at[5]),
    ]
    wo_copy = pltpu.make_async_copy(wo_hbm, wo_v, sem_in.at[6])

    srcs = [r.bitcast(jnp.uint32) for r in (wq_hbm, wk_hbm, wv_hbm)]

    def pair_copy(m, j):
        return pltpu.make_async_copy(srcs[m].at[:, j, :], stage_v.at[m * n_pair + j],
                                     sem_w.at[m * n_pair + j])

    for c in small:
        c.start()
    for j in range(n_pair):
        for m in range(3):
            pair_copy(m, j).start()
    wo_copy.start()
    for c in small:
        c.wait()

    pairs_per_chunk = n_pair // n_chunk

    def mlp_chunk(i, carry):
        r0 = pl.multiple_of(i * _MC, _MC)
        xc = x_v[pl.ds(r0, _MC), :]
        gate = jax.nn.sigmoid(jnp.sum(xc.astype(_F32) * gw_v[...].astype(_F32), axis=-1, keepdims=True))
        gg = _dot(xc, wg_v[...])
        uu = _dot(xc, wu_v[...])
        hh = (jax.nn.gelu(gg, approximate=True) * uu).astype(_BF16)
        bb = _dot(hh, wd_v[...])
        b_v[pl.ds(r0, _MC), :] = (1.0 - gate) * bb
        g_v[pl.ds(r0, _MC), :] = jnp.broadcast_to(gate, (_MC, 128))
        for jj in range(pairs_per_chunk):
            j = i * pairs_per_chunk + jj
            for m in range(3):
                pair_copy(m, j).wait()
                w = stage_v[m * n_pair + j]
                lo = lax.bitcast_convert_type(w << 16, _F32).astype(_BF16)
                hi = lax.bitcast_convert_type(w & jnp.uint32(0xFFFF0000), _F32).astype(_BF16)
                w_v[m, 2 * j] = lo
                w_v[m, 2 * j + 1] = hi
        return carry

    lax.fori_loop(0, n_chunk, mlp_chunk, 0)
    wo_copy.wait()

    row = lax.broadcasted_iota(jnp.int32, (L, L), 0)
    col = lax.broadcasted_iota(jnp.int32, (L, L), 1)
    mask = (row < M) | (row >= col)

    def proj(h, m):
        w = jnp.concatenate([w_v[m, hd] for hd in range(n_heads)], axis=1)
        return _dot(h, w)

    def step(s, mem):
        r0 = pl.multiple_of(s * seg, seg)
        xs = x_v[pl.ds(r0, seg), :].astype(_F32)
        h = jnp.concatenate([mem, xs], axis=0)
        q = proj(h, 0)
        k = proj(h, 1).astype(_BF16)
        sc = []
        for hd in range(n_heads):
            sl = slice(hd * Dh, (hd + 1) * Dh)
            sc.append(lax.dot_general(q[:, sl], k[:, sl], (((1,), (1,)), ((), ())),
                                      preferred_element_type=_F32))
        v = proj(h, 2).astype(_BF16)
        os_ = []
        for hd in range(n_heads):
            sl = slice(hd * Dh, (hd + 1) * Dh)
            t = jnp.where(mask, sc[hd] * scale, -1000000000.0)
            e = jnp.exp(t - jnp.max(t, axis=-1, keepdims=True))
            p = e / jnp.sum(e, axis=-1, keepdims=True)
            os_.append(_dot(p, v[:, sl]))
        o = jnp.concatenate(os_, axis=1)
        a = _dot(o, wo_v[...])
        g = g_v[pl.ds(r0, seg), :]
        g = jnp.concatenate([g] * (Dm // 128), axis=1)
        o_v[pl.ds(r0, seg), :] = (g * a[M:] + b_v[pl.ds(r0, seg), :]).astype(o_v.dtype)
        return a[:M].astype(_BF16).astype(_F32)

    lax.fori_loop(0, n_seg, step, mem_v[...].astype(_F32))
    oc = pltpu.make_async_copy(o_v, out_hbm, sem_out.at[0])
    oc.start()
    oc.wait()


@functools.partial(jax.jit, static_argnames=("A_seg_len",))
def pallas_gated_mix__memory_aug_recurrent_mem_tr__glu_gated_geglu__prompt_kernel(
    A_x, A_mem0, A_Wq, A_Wk, A_Wv, A_Wo, A_seg_len, B_x, B_w_gate, B_w_up, B_w_down, gate_w,
):
    del B_x
    B, S, Dm = A_x.shape
    _, H, Dh = A_Wq.shape
    M = A_mem0.shape[1]
    Df = B_w_gate.shape[1]
    assert B == 1
    any_spec = pl.BlockSpec(memory_space=pl.ANY)
    out = pl.pallas_call(
        functools.partial(_kernel, seg=int(A_seg_len), n_heads=H),
        out_shape=jax.ShapeDtypeStruct((S, Dm), A_x.dtype),
        in_specs=[any_spec] * 10,
        out_specs=any_spec,
        scratch_shapes=[
            pltpu.VMEM((S, Dm), _BF16),
            pltpu.VMEM((M, Dm), _BF16),
            pltpu.VMEM((1, Dm), _BF16),
            pltpu.VMEM((Dm, Df), _BF16),
            pltpu.VMEM((Dm, Df), _BF16),
            pltpu.VMEM((Df, Dm), _BF16),
            pltpu.VMEM((3 * H // 2, Dm, Dh), jnp.uint32),
            pltpu.VMEM((3, H, Dm, Dh), _BF16),
            pltpu.VMEM((H * Dh, Dm), _BF16),
            pltpu.VMEM((S, Dm), _F32),
            pltpu.VMEM((S, 128), _F32),
            pltpu.VMEM((S, Dm), A_x.dtype),
            pltpu.SemaphoreType.DMA((7,)),
            pltpu.SemaphoreType.DMA((3 * H // 2,)),
            pltpu.SemaphoreType.DMA((1,)),
        ],
        compiler_params=pltpu.CompilerParams(vmem_limit_bytes=110 * 2**20),
    )(A_x.reshape(S, Dm), A_mem0.reshape(M, Dm), A_Wq, A_Wk, A_Wv, A_Wo.reshape(H * Dh, Dm),
      B_w_gate, B_w_up, B_w_down, gate_w.reshape(1, Dm))
    return out.reshape(B, S, Dm)
```

```python
import functools

import jax
import jax.numpy as jnp
from jax import lax
import jax.experimental.pallas as pl
import jax.experimental.pallas.tpu as pltpu

_F32 = jnp.float32
_BF16 = jnp.bfloat16
_OUT_CHUNKS = 16
_MC = 512


def _dot(a, b):
    return jnp.dot(a, b, preferred_element_type=_F32)


def _dot_t(a, b):
    return lax.dot_general(a, b, (((1,), (1,)), ((), ())), preferred_element_type=_F32)


def _kernel(x_hbm, mem_hbm, wq_hbm, wk_hbm, wv_hbm, wo_hbm, wg_hbm, wu_hbm, wd_hbm, gw_hbm,
            out_hbm,
            x_v, mem_v, gw_v, wg_v, wu_v, wt_v, wd_v, stage_v, w_v, wo_v, b_v, g_v, o_v,
            sem_in, sem_w, sem_out, *, seg, n_heads):
    S, Dm = x_v.shape
    M = mem_v.shape[0]
    Dh = stage_v.shape[2]
    L = M + seg
    n_seg = S // seg
    n_pair = n_heads // 2
    n_chunk = S // _MC
    scale = Dh ** (-0.5)

    Df = wd_v.shape[0]
    Fm = wg_v.shape[0]
    Ft = Df - Fm
    first = [
        pltpu.make_async_copy(x_hbm.at[pl.ds(0, _MC)], x_v.at[pl.ds(0, _MC)], sem_in.at[0]),
        pltpu.make_async_copy(wg_hbm.at[pl.ds(0, Fm)], wg_v, sem_in.at[1]),
        pltpu.make_async_copy(gw_hbm, gw_v, sem_in.at[2]),
    ]
    second = [
        pltpu.make_async_copy(wu_hbm.at[pl.ds(0, Fm)], wu_v, sem_in.at[3]),
        pltpu.make_async_copy(wg_hbm.at[pl.ds(Fm, Ft)], wt_v.at[pl.ds(0, Ft)], sem_in.at[4]),
        pltpu.make_async_copy(wu_hbm.at[pl.ds(Fm, Ft)], wt_v.at[pl.ds(Ft, Ft)], sem_in.at[5]),
    ]
    third = [
        pltpu.make_async_copy(wd_hbm, wd_v, sem_in.at[7]),
        pltpu.make_async_copy(x_hbm.at[pl.ds(_MC, S - _MC)], x_v.at[pl.ds(_MC, S - _MC)], sem_in.at[8]),
        pltpu.make_async_copy(mem_hbm, mem_v, sem_in.at[9]),
    ]
    wo_copy = pltpu.make_async_copy(wo_hbm, wo_v, sem_in.at[6])

    srcs = [r.bitcast(jnp.uint32) for r in (wq_hbm, wk_hbm, wv_hbm)]

    def pair_copy(m, j):
        return pltpu.make_async_copy(srcs[m].at[:, j, :], stage_v.at[m * n_pair + j],
                                     sem_w.at[m * n_pair + j])

    for c in first + second + third:
        c.start()
    pairs_per_chunk = n_pair // n_chunk

    def start_pairs(i):
        for jj in range(pairs_per_chunk):
            for m in range(3):
                pair_copy(m, i * pairs_per_chunk + jj).start()

    for c in first:
        c.wait()

    def mlp_chunk(i, carry):
        r0 = pl.multiple_of(i * _MC, _MC)

        xc = x_v[pl.ds(r0, _MC), :]
        gate = jax.nn.sigmoid(jnp.sum(xc.astype(_F32) * gw_v[...].astype(_F32), axis=-1, keepdims=True))
        gg = jax.nn.gelu(_dot_t(xc, wg_v[...]), approximate=True)

        @pl.when(i == 0)
        def _():
            for c in second:
                c.wait()
            start_pairs(0)
            start_pairs(1)

        hh = (gg * _dot_t(xc, wu_v[...])).astype(_BF16)
        tt = _dot_t(xc, wt_v[...])
        ht = (jax.nn.gelu(tt, approximate=True) * pltpu.roll(tt, Ft, 1))[:, :Ft].astype(_BF16)

        @pl.when(i == 0)
        def _():
            for c in third:
                c.wait()

        @pl.when(i + 2 < n_chunk)
        def _():
            start_pairs(i + 2)

        @pl.when(i + 2 == n_chunk)
        def _():
            wo_copy.start()

        bb = _dot(hh, wd_v[pl.ds(0, Fm), :]) + _dot(ht, wd_v[pl.ds(Fm, Ft), :])
        b_v[pl.ds(r0, _MC), :] = (1.0 - gate) * bb
        g_v[pl.ds(r0, _MC), :] = jnp.broadcast_to(gate, (_MC, 128))
        for jj in range(pairs_per_chunk):
            j = i * pairs_per_chunk + jj
            for m in range(3):
                pair_copy(m, j).wait()
                w = stage_v[m * n_pair + j]
                lo = lax.bitcast_convert_type(w << 16, _F32).astype(_BF16)
                hi = lax.bitcast_convert_type(w & jnp.uint32(0xFFFF0000), _F32).astype(_BF16)
                w_v[m, 2 * j] = lo
                w_v[m, 2 * j + 1] = hi
        return carry

    lax.fori_loop(0, n_chunk, mlp_chunk, 0)
    wo_copy.wait()

    row = lax.broadcasted_iota(jnp.int32, (L, L), 0)
    col = lax.broadcasted_iota(jnp.int32, (L, L), 1)
    mask = (row < M) | (row >= col)

    def proj(h, m):
        w = jnp.concatenate([w_v[m, hd] for hd in range(n_heads)], axis=1)
        return _dot(h, w)

    def step(s, mem):
        r0 = pl.multiple_of(s * seg, seg)
        xs = x_v[pl.ds(r0, seg), :].astype(_F32)
        h = jnp.concatenate([mem, xs], axis=0)
        q = proj(h, 0)
        k = proj(h, 1).astype(_BF16)
        sc = []
        for hd in range(n_heads):
            sl = slice(hd * Dh, (hd + 1) * Dh)
            sc.append(lax.dot_general(q[:, sl], k[:, sl], (((1,), (1,)), ((), ())),
                                      preferred_element_type=_F32))
        v = proj(h, 2).astype(_BF16)
        os_ = []
        for hd in range(n_heads):
            sl = slice(hd * Dh, (hd + 1) * Dh)
            t = jnp.where(mask, sc[hd] * scale, -1000000000.0)
            e = jnp.exp(t - jnp.max(t, axis=-1, keepdims=True))
            p = e / jnp.sum(e, axis=-1, keepdims=True)
            os_.append(_dot(p, v[:, sl]))
        o = jnp.concatenate(os_, axis=1)
        a = _dot(o, wo_v[...])
        g = g_v[pl.ds(r0, seg), :]
        g = jnp.concatenate([g] * (Dm // 128), axis=1)
        o_v[pl.ds(r0, seg), :] = (g * a[M:] + b_v[pl.ds(r0, seg), :]).astype(o_v.dtype)
        return a[:M].astype(_BF16).astype(_F32)

    rows = S // _OUT_CHUNKS
    steps = n_seg // _OUT_CHUNKS

    def out_copy(c):
        r0 = pl.multiple_of(c * rows, rows)
        return pltpu.make_async_copy(o_v.at[pl.ds(r0, rows)], out_hbm.at[pl.ds(r0, rows)], sem_out.at[c])

    def step_group(c, mem):
        for u in range(steps):
            mem = step(c * steps + u, mem)
        out_copy(c).start()
        return mem

    lax.fori_loop(0, _OUT_CHUNKS, step_group, mem_v[...].astype(_F32))
    for c in range(_OUT_CHUNKS):
        out_copy(c).wait()


@functools.partial(jax.jit, static_argnames=("A_seg_len",))
def pallas_gated_mix__memory_aug_recurrent_mem_tr__glu_gated_geglu__prompt_kernel(
    A_x, A_mem0, A_Wq, A_Wk, A_Wv, A_Wo, A_seg_len, B_x, B_w_gate, B_w_up, B_w_down, gate_w,
):
    del B_x
    B, S, Dm = A_x.shape
    _, H, Dh = A_Wq.shape
    M = A_mem0.shape[1]
    Df = B_w_gate.shape[1]
    Fm = Df // 128 * 128
    assert B == 1 and 2 * (Df - Fm) == 128
    any_spec = pl.BlockSpec(memory_space=pltpu.HBM)
    out = pl.pallas_call(
        functools.partial(_kernel, seg=int(A_seg_len), n_heads=H),
        out_shape=jax.ShapeDtypeStruct((S, Dm), A_x.dtype),
        in_specs=[any_spec] * 10,
        out_specs=any_spec,
        scratch_shapes=[
            pltpu.VMEM((S, Dm), _BF16),
            pltpu.VMEM((M, Dm), _BF16),
            pltpu.VMEM((1, Dm), _BF16),
            pltpu.VMEM((Fm, Dm), _BF16),
            pltpu.VMEM((Fm, Dm), _BF16),
            pltpu.VMEM((2 * (Df - Fm), Dm), _BF16),
            pltpu.VMEM((Df, Dm), _BF16),
            pltpu.VMEM((3 * H // 2, Dm, Dh), jnp.uint32),
            pltpu.VMEM((3, H, Dm, Dh), _BF16),
            pltpu.VMEM((H * Dh, Dm), _BF16),
            pltpu.VMEM((S, Dm), _F32),
            pltpu.VMEM((S, 128), _F32),
            pltpu.VMEM((S, Dm), A_x.dtype),
            pltpu.SemaphoreType.DMA((10,)),
            pltpu.SemaphoreType.DMA((3 * H // 2,)),
            pltpu.SemaphoreType.DMA((_OUT_CHUNKS,)),
        ],
        compiler_params=pltpu.CompilerParams(vmem_limit_bytes=110 * 2**20),
    )(A_x.reshape(S, Dm), A_mem0.reshape(M, Dm), A_Wq, A_Wk, A_Wv, A_Wo.reshape(H * Dh, Dm),
      B_w_gate.T, B_w_up.T, B_w_down, gate_w.reshape(1, Dm))
    return out.reshape(B, S, Dm)
```
